```python
import os as _os
_os.environ.setdefault("JAX_PLATFORMS", "cpu")
import jax
import jax.numpy as jnp

def _softmax(x, axis=-1):
    return jax.nn.softmax(x, axis=axis)
def _gelu(x):
    return jax.nn.gelu(x, approximate=True)
def _silu(x):
    return jax.nn.silu(x)
def _sigmoid(x):
    return jax.nn.sigmoid(x)
def _layernorm(x, axis=-1, eps=1e-5):
    m = jnp.mean(x, axis=axis, keepdims=True)
    v = jnp.var(x, axis=axis, keepdims=True)
    return (x - m) / jnp.sqrt(v + eps)
def _scatter_add(tgt, idx, src, axis=0):
    return tgt.at[idx].add(src)
def _segment_sum(src, seg, n):
    return jax.ops.segment_sum(src, seg, n)
class _Rng:
    def __init__(self, key):
        self._k = key
    def _next(self):
        self._k, sub = jax.random.split(self._k)
        return sub
    def normal(self, shape):
        return jax.random.normal(self._next(), shape, dtype=jnp.bfloat16)
    def randint(self, lo, hi, shape):
        return jax.random.randint(self._next(), shape, lo, hi, dtype=jnp.int32)
    def uniform(self, shape, lo=0.0, hi=1.0):
        return jax.random.uniform(self._next(), shape, jnp.bfloat16, lo, hi)
    def permutation(self, n):
        return jax.random.permutation(self._next(), n)


kernel_name = 'gated_mix__gqa_block_cached__dense_activation_squared_relu__decode'

def setup_inputs():
    _rng = _Rng(jax.random.key(int.from_bytes(__import__("os").urandom(4), "little")))
    _w = (lambda a: (lambda t: t.astype(jnp.bfloat16) if jnp.issubdtype(t.dtype, jnp.floating) else t)(jnp.asarray(a)))
    def _A_setup():
        B, Sq, D = 4, 1, 512
        Hq, Hkv, Sk, Dh = 32, 8, 4096, 128
        assert Hq % Hkv == 0, (Hq, Hkv)
        return {
            "x": _w((lambda *s: _rng.normal(s) * 0.05)(B, Sq, D)),
            "k_cache": _w((lambda *s: _rng.normal(s) * 3.2)(B, Hkv, Sk, Dh)),
            "v_cache": _w((lambda *s: _rng.normal(s) * 1.6)(B, Hkv, Sk, Dh)),
            "wq": _w((lambda *s: _rng.normal(s) * 3.2)(D, Hq * Dh) * (D ** -0.5)),
            "wo": _w((lambda *s: _rng.normal(s) * 1.6)(Hq * Dh, D) * ((Hq * Dh) ** -0.5)),
        }
    _A_in = _A_setup()

    def _B_setup():
        B, S, D, F = 4, 1, 512, 1792
        return {
            "x": _w((lambda *s: _rng.normal(s) * 0.05)(B, S, D)),
            "w1": _w((lambda *s: _rng.normal(s) * 0.1)(D, F)),
            "b1": _w((lambda *s: _rng.normal(s) * 0.05)(F)),
            "w2": _w((lambda *s: _rng.normal(s) * 0.05)(F, D)),
            "b2": _w((lambda *s: _rng.normal(s) * 0.05)(D)),
        }
    _B_in = _B_setup()

    return {
        "A_x": _A_in["x"],
        "A_k_cache": _A_in["k_cache"],
        "A_v_cache": _A_in["v_cache"],
        "A_wq": _A_in["wq"],
        "A_wo": _A_in["wo"],
        "B_x": _B_in["x"],
        "B_w1": _B_in["w1"],
        "B_b1": _B_in["b1"],
        "B_w2": _B_in["w2"],
        "B_b2": _B_in["b2"],
        "gate_w": _w((lambda *s: _rng.normal(s) * 0.05)(512) * 16.0),
    }

def reference(A_x, A_k_cache, A_v_cache, A_wq, A_wo, B_x, B_w1, B_b1, B_w2, B_b2, gate_w):
    def _A_ref(x, k_cache, v_cache, wq, wo):
        B, Sq, D = x.shape
        Hq, Dh = 32, 128
        Hkv = k_cache.shape[1]
        rep = Hq // Hkv
        q = (lambda x, *d: x.transpose(*d))((x @ wq).reshape(B, Sq, Hq, Dh), 0, 2, 1, 3)
        k = jnp.repeat(k_cache, rep, axis=1)
        v = jnp.repeat(v_cache, rep, axis=1)
        scores = jnp.einsum("bhqd,bhkd->bhqk", q, k) * (Dh ** -0.5)
        p = _softmax(scores, axis=-1)
        o = jnp.einsum("bhqk,bhkd->bhqd", p, v)
        return (lambda x, *d: x.transpose(*d))(o, 0, 2, 1, 3).reshape(B, Sq, Hq * Dh) @ wo

    def _B_ref(x, w1, b1, w2, b2):
        h = jnp.einsum("bsd,df->bsf", x, w1) + b1
        zero = jnp.zeros_like(h)
        r = jnp.where(h > zero, h, zero)
        h = r * r
        out = jnp.einsum("bsf,fd->bsd", h, w2) + b2
        return out

    x = A_x
    g = _sigmoid((x * gate_w).sum(-1, keepdims=True))
    a = _A_ref(x, A_k_cache, A_v_cache, A_wq, A_wo)
    b = _B_ref(x, B_w1, B_b1, B_w2, B_b2)
    return g * a + (1 - g) * b
```

```python
import jax
import jax.numpy as jnp
from jax import lax
import jax.experimental.pallas as pl
import jax.experimental.pallas.tpu as pltpu


@jax.jit
def pallas_gated_mix__gqa_block_cached__dense_activation_squared_relu__decode_kernel(
    A_x: jax.Array,
    A_k_cache: jax.Array,
    A_v_cache: jax.Array,
    A_wq: jax.Array,
    A_wo: jax.Array,
    B_x: jax.Array,
    B_w1: jax.Array,
    B_b1: jax.Array,
    B_w2: jax.Array,
    B_b2: jax.Array,
    gate_w: jax.Array,
):
    del B_x
    B, _, D = A_x.shape
    _, Hkv, Sk, Dh = A_k_cache.shape
    Hq = A_wq.shape[1] // Dh
    F = B_w1.shape[1]
    rep = Hq // Hkv
    scale = Dh ** -0.5
    f32, bf16 = jnp.float32, jnp.bfloat16

    def kern(x_ref, k_ref, v_ref, wq_ref, wo_ref, w1_ref, b1_ref, w2_ref, b2_ref, gw_ref, o_ref,
             q_s, o_s, ffn_s):
        b = pl.program_id(0)
        h = pl.program_id(1)

        @pl.when((b == 0) & (h == 0))
        def _():
            x = x_ref[...]
            q = jnp.dot(x, wq_ref[...], preferred_element_type=f32)
            q = q.astype(bf16).astype(f32)
            for j in range(Hq):
                q_s[pl.ds(j, B, stride=Hq), :] = q[:, j * Dh:(j + 1) * Dh]
            hh = jnp.dot(x, w1_ref[...], preferred_element_type=f32).astype(bf16) + b1_ref[...].reshape(1, F)
            hh = hh.astype(f32)
            r = jnp.where(hh > 0, hh, 0.0)
            h2 = (r * r).astype(bf16)
            ffn = jnp.dot(h2, w2_ref[...], preferred_element_type=f32).astype(bf16) + b2_ref[...].reshape(1, D)
            ffn_s[...] = ffn.astype(f32)

        row0 = b * Hq + h * rep
        q = q_s[pl.ds(row0, rep), :].astype(bf16)
        s = lax.dot_general(q, k_ref[0, 0], (((1,), (1,)), ((), ())), preferred_element_type=f32)
        s = s * scale
        m = jnp.max(s, axis=-1, keepdims=True)
        e = jnp.exp(s - m)
        l = jnp.sum(e, axis=-1, keepdims=True)
        o = jnp.dot(e.astype(bf16), v_ref[0, 0], preferred_element_type=f32)
        o_s[pl.ds(row0, rep), :] = o / l

        @pl.when((b == B - 1) & (h == Hkv - 1))
        def _():
            acc = jnp.zeros((B, D), f32)
            for j in range(Hq):
                oj = o_s[pl.ds(j, B, stride=Hq), :].astype(bf16)
                acc += jnp.dot(oj, wo_ref[j * Dh:(j + 1) * Dh, :], preferred_element_type=f32)
            x = x_ref[...].astype(f32)
            gl = jnp.sum(x * gw_ref[...].reshape(1, D).astype(f32), axis=-1, keepdims=True)
            gate = jax.nn.sigmoid(gl)
            o_ref[...] = (gate * acc + (1 - gate) * ffn_s[...]).astype(o_ref.dtype)

    one = dict(pipeline_mode=pl.Buffered(1))
    full = lambda shape: pl.BlockSpec(shape, lambda b, h: (0,) * len(shape), **one)
    out = pl.pallas_call(
        kern,
        out_shape=jax.ShapeDtypeStruct((B, D), bf16),
        grid=(B, Hkv),
        in_specs=[full((B, D)),
                  pl.BlockSpec((1, 1, Sk, Dh), lambda b, h: (b, h, 0, 0)),
                  pl.BlockSpec((1, 1, Sk, Dh), lambda b, h: (b, h, 0, 0)),
                  full((D, Hq * Dh)), full((Hq * Dh, D)), full((D, F)), full((F,)), full((F, D)), full((D,)), full((D,))],
        out_specs=pl.BlockSpec((B, D), lambda b, h: (0, 0)),
        scratch_shapes=[pltpu.VMEM((B * Hq, Dh), f32), pltpu.VMEM((B * Hq, Dh), f32), pltpu.VMEM((B, D), f32)],
        compiler_params=pltpu.CompilerParams(vmem_limit_bytes=100 * 1024 * 1024,
                                             dimension_semantics=("arbitrary", "arbitrary")),
    )(A_x.reshape(B, D), A_k_cache, A_v_cache, A_wq, A_wo, B_w1, B_b1, B_w2, B_b2, gate_w)
    return out.reshape(B, 1, D)
```

```python
import jax
import jax.numpy as jnp
from jax import lax
import jax.experimental.pallas as pl
import jax.experimental.pallas.tpu as pltpu

NS = 3
WO_CHUNKS = (512,) * 7 + (256, 128, 128)


@jax.jit
def pallas_gated_mix__gqa_block_cached__dense_activation_squared_relu__decode_kernel(
    A_x: jax.Array,
    A_k_cache: jax.Array,
    A_v_cache: jax.Array,
    A_wq: jax.Array,
    A_wo: jax.Array,
    B_x: jax.Array,
    B_w1: jax.Array,
    B_b1: jax.Array,
    B_w2: jax.Array,
    B_b2: jax.Array,
    gate_w: jax.Array,
):
    del B_x
    B, _, D = A_x.shape
    _, Hkv, Sk, Dh = A_k_cache.shape
    Hq = A_wq.shape[1] // Dh
    F = B_w1.shape[1]
    rep = Hq // Hkv
    NH = B * Hkv
    scale = Dh ** -0.5
    f32, bf16 = jnp.float32, jnp.bfloat16
    NW = len(WO_CHUNKS)
    assert sum(WO_CHUNKS) == Hq * Dh and all(c % Dh == 0 for c in WO_CHUNKS)
    wo_off = [sum(WO_CHUNKS[:c]) for c in range(NW)]

    def stream(x_hbm, k_hbm, v_hbm, wq_hbm, wo_hbm, w1_hbm, b1_hbm, w2_hbm, b2_hbm, gw_hbm, gate_base,
               x_v, wq_v, w1_v, b1_v, w2_v, b2_v, gw_v, kb, vb, wo_v, q_s, o_s, sem):
        pre = [(x_hbm, x_v), (wq_hbm, wq_v), (gw_hbm, gw_v), (b1_hbm, b1_v), (b2_hbm, b2_v),
               (w1_hbm, w1_v), (w2_hbm, w2_v)]
        pre_c = [pltpu.make_async_copy(s, d, sem.at[0]) for s, d in pre]

        def head_c(i):
            sm = sem.at[(i + 1) % NS]
            return (pltpu.make_async_copy(k_hbm.at[i // Hkv, i % Hkv], kb.at[i], sm),
                    pltpu.make_async_copy(v_hbm.at[i // Hkv, i % Hkv], vb.at[i], sm))

        def wo_c(c):
            sl = pl.ds(wo_off[c], WO_CHUNKS[c])
            return pltpu.make_async_copy(wo_hbm.at[sl], wo_v.at[sl], sem.at[(NH + 1 + c) % NS])

        for cp in pre_c:
            cp.start()
        for i in range(NS - 1):
            for cp in head_c(i):
                cp.start()
        for cp in pre_c:
            cp.wait()
        for cp in head_c(NS - 1):
            cp.start()

        x = x_v[...]
        q = jnp.dot(x, wq_v[...], preferred_element_type=f32).astype(bf16).astype(f32)
        for j in range(Hq):
            q_s[pl.ds(j, B, stride=Hq), :] = q[:, j * Dh:(j + 1) * Dh]

        gl = jnp.sum(x.astype(f32) * gw_v[...].reshape(1, D).astype(f32), axis=-1, keepdims=True)
        gate = jax.nn.sigmoid(gl)
        hh = jnp.dot(x, w1_v[...], preferred_element_type=f32).astype(bf16) + b1_v[...].reshape(1, F)
        hh = hh.astype(f32)
        r = jnp.where(hh > 0, hh, 0.0)
        h2 = (r * r).astype(bf16)
        ffn = jnp.dot(h2, w2_v[...], preferred_element_type=f32).astype(bf16) + b2_v[...].reshape(1, D)
        base = (1 - gate) * ffn.astype(f32)

        def head_step(i, carry):
            for cp in head_c(i):
                cp.wait()

            @pl.when(i + NS < NH)
            def _():
                for cp in head_c(i + NS):
                    cp.start()

            for c in range(NS):
                @pl.when(i + NS == NH + c)
                def _():
                    wo_c(c).start()

            row0 = pl.multiple_of(i * rep, rep)
            qq = q_s[pl.ds(row0, rep), :].astype(bf16)
            s = lax.dot_general(qq, kb[i], (((1,), (1,)), ((), ())), preferred_element_type=f32)
            s = s * scale
            m = jnp.max(s, axis=-1, keepdims=True)
            e = jnp.exp(s - m)
            l = jnp.sum(e, axis=-1, keepdims=True)
            o = jnp.dot(e.astype(bf16), vb[i], preferred_element_type=f32)
            o_s[pl.ds(row0, rep), :] = o / l
            return carry

        lax.fori_loop(0, NH, head_step, 0)

        acc = jnp.zeros((B, D), f32)
        for c in range(NW):
            wo_c(c).wait()
            if c + NS < NW:
                wo_c(c + NS).start()
            for jj in range(WO_CHUNKS[c] // Dh):
                j = wo_off[c] // Dh + jj
                oj = o_s[pl.ds(j, B, stride=Hq), :].astype(bf16)
                acc += jnp.dot(oj, wo_v[pl.ds(j * Dh, Dh), :], preferred_element_type=f32)
        gate_base(gate * acc + base)

    def kern(*refs):
        o_ref = refs[10]
        rest = refs[:10] + (lambda val: o_ref.__setitem__(Ellipsis, val.astype(o_ref.dtype)),) + refs[11:]
        pl.run_scoped(lambda sem: stream(*rest, sem), pltpu.SemaphoreType.DMA((NS,)))

    out = pl.pallas_call(
        kern,
        out_shape=jax.ShapeDtypeStruct((B, D), bf16),
        in_specs=[pl.BlockSpec(memory_space=pl.ANY)] * 10,
        out_specs=pl.BlockSpec(memory_space=pltpu.VMEM),
        scratch_shapes=[
            pltpu.VMEM((B, D), bf16),
            pltpu.VMEM((D, Hq * Dh), bf16),
            pltpu.VMEM((D, F), bf16),
            pltpu.VMEM((F,), bf16),
            pltpu.VMEM((F, D), bf16),
            pltpu.VMEM((D,), bf16),
            pltpu.VMEM((D,), bf16),
            pltpu.VMEM((NH, Sk, Dh), bf16),
            pltpu.VMEM((NH, Sk, Dh), bf16),
            pltpu.VMEM((Hq * Dh, D), bf16),
            pltpu.VMEM((B * Hq, Dh), f32),
            pltpu.VMEM((B * Hq, Dh), f32),
        ],
        compiler_params=pltpu.CompilerParams(vmem_limit_bytes=100 * 1024 * 1024),
    )(A_x.reshape(B, D), A_k_cache, A_v_cache, A_wq, A_wo, B_w1, B_b1, B_w2, B_b2, gate_w)
    return out.reshape(B, 1, D)
```

```python
import jax
import jax.numpy as jnp
from jax import lax
import jax.experimental.pallas as pl
import jax.experimental.pallas.tpu as pltpu

NS = 3
WO_CHUNKS = (512,) * 7 + (256, 128, 128)


@jax.jit
def pallas_gated_mix__gqa_block_cached__dense_activation_squared_relu__decode_kernel(
    A_x: jax.Array,
    A_k_cache: jax.Array,
    A_v_cache: jax.Array,
    A_wq: jax.Array,
    A_wo: jax.Array,
    B_x: jax.Array,
    B_w1: jax.Array,
    B_b1: jax.Array,
    B_w2: jax.Array,
    B_b2: jax.Array,
    gate_w: jax.Array,
):
    del B_x
    B, _, D = A_x.shape
    _, Hkv, Sk, Dh = A_k_cache.shape
    Hq = A_wq.shape[1] // Dh
    F = B_w1.shape[1]
    rep = Hq // Hkv
    NH = B * Hkv
    scale = Dh ** -0.5
    f32, bf16 = jnp.float32, jnp.bfloat16
    NW = len(WO_CHUNKS)
    assert NS <= NW and sum(WO_CHUNKS) == Hq * Dh and all(c % Dh == 0 for c in WO_CHUNKS)
    wo_off = [sum(WO_CHUNKS[:c]) for c in range(NW)]

    def kernel(x_hbm, k_hbm, v_hbm, wq_hbm, wo_hbm, w1_hbm, b1_hbm, w2_hbm, b2_hbm, gw_hbm, o_ref,
               x_v, wq_v, w1_v, b1_v, w2_v, b2_v, gw_v, k_v, v_v, wo_v, q_s, o_s):

        def run(sem):
            pre_c = [pltpu.make_async_copy(src, dst, sem.at[0]) for src, dst in (
                (x_hbm, x_v), (wq_hbm, wq_v), (gw_hbm, gw_v), (b1_hbm, b1_v), (b2_hbm, b2_v),
                (w1_hbm, w1_v), (w2_hbm, w2_v))]

            def head_c(i):
                b, h, sm = i // Hkv, i % Hkv, sem.at[(i + 1) % NS]
                return (pltpu.make_async_copy(k_hbm.at[b, h], k_v.at[i], sm),
                        pltpu.make_async_copy(v_hbm.at[b, h], v_v.at[i], sm))

            def wo_c(c):
                rows = pl.ds(wo_off[c], WO_CHUNKS[c])
                return pltpu.make_async_copy(wo_hbm.at[rows], wo_v.at[rows],
                                             sem.at[(NH + 1 + c) % NS])

            for cp in pre_c:
                cp.start()
            for i in range(NS - 1):
                for cp in head_c(i):
                    cp.start()
            for cp in pre_c:
                cp.wait()
            for cp in head_c(NS - 1):
                cp.start()

            x = x_v[...]
            q = jnp.dot(x, wq_v[...], preferred_element_type=f32).astype(bf16).astype(f32)
            for j in range(Hq):
                q_s[pl.ds(j, B, stride=Hq), :] = q[:, j * Dh:(j + 1) * Dh]

            logit = jnp.sum(x.astype(f32) * gw_v[...].reshape(1, D).astype(f32),
                            axis=-1, keepdims=True)
            gate = jax.nn.sigmoid(logit)
            hid = jnp.dot(x, w1_v[...], preferred_element_type=f32).astype(bf16)
            hid = (hid + b1_v[...].reshape(1, F)).astype(f32)
            relu = jnp.where(hid > 0, hid, 0.0)
            act = (relu * relu).astype(bf16)
            ffn = jnp.dot(act, w2_v[...], preferred_element_type=f32).astype(bf16)
            ffn = (ffn + b2_v[...].reshape(1, D)).astype(f32)
            base = (1 - gate) * ffn

            def head_step(i, carry):
                for cp in head_c(i):
                    cp.wait()

                @pl.when(i + NS < NH)
                def _():
                    for cp in head_c(i + NS):
                        cp.start()

                for c in range(NS):
                    @pl.when(i + NS == NH + c)
                    def _():
                        wo_c(c).start()

                row0 = pl.multiple_of(i * rep, rep)
                qh = q_s[pl.ds(row0, rep), :].astype(bf16)
                s = lax.dot_general(qh, k_v[i], (((1,), (1,)), ((), ())),
                                    preferred_element_type=f32) * scale
                m = jnp.max(s, axis=-1, keepdims=True)
                e = jnp.exp(s - m)
                l = jnp.sum(e, axis=-1, keepdims=True)
                o = jnp.dot(e.astype(bf16), v_v[i], preferred_element_type=f32)
                o_s[pl.ds(row0, rep), :] = o / l
                return carry

            lax.fori_loop(0, NH, head_step, 0)

            acc = jnp.zeros((B, D), f32)
            for c in range(NW):
                wo_c(c).wait()
                if c + NS < NW:
                    wo_c(c + NS).start()
                for j in range(wo_off[c] // Dh, (wo_off[c] + WO_CHUNKS[c]) // Dh):
                    oj = o_s[pl.ds(j, B, stride=Hq), :].astype(bf16)
                    acc += jnp.dot(oj, wo_v[pl.ds(j * Dh, Dh), :], preferred_element_type=f32)
            o_ref[...] = (gate * acc + base).astype(o_ref.dtype)

        pl.run_scoped(run, pltpu.SemaphoreType.DMA((NS,)))

    out = pl.pallas_call(
        kernel,
        out_shape=jax.ShapeDtypeStruct((B, D), bf16),
        in_specs=[pl.BlockSpec(memory_space=pl.ANY)] * 10,
        out_specs=pl.BlockSpec(memory_space=pltpu.VMEM),
        scratch_shapes=[
            pltpu.VMEM((B, D), bf16),
            pltpu.VMEM((D, Hq * Dh), bf16),
            pltpu.VMEM((D, F), bf16),
            pltpu.VMEM((F,), bf16),
            pltpu.VMEM((F, D), bf16),
            pltpu.VMEM((D,), bf16),
            pltpu.VMEM((D,), bf16),
            pltpu.VMEM((NH, Sk, Dh), bf16),
            pltpu.VMEM((NH, Sk, Dh), bf16),
            pltpu.VMEM((Hq * Dh, D), bf16),
            pltpu.VMEM((B * Hq, Dh), f32),
            pltpu.VMEM((B * Hq, Dh), f32),
        ],
        compiler_params=pltpu.CompilerParams(vmem_limit_bytes=100 * 1024 * 1024),
    )(A_x.reshape(B, D), A_k_cache, A_v_cache, A_wq, A_wo, B_w1, B_b1, B_w2, B_b2, gate_w)
    return out.reshape(B, 1, D)
```
